```python
import os as _os
_os.environ.setdefault("JAX_PLATFORMS", "cpu")
import jax
import jax.numpy as jnp

def _softmax(x, axis=-1):
    return jax.nn.softmax(x, axis=axis)
def _gelu(x):
    return jax.nn.gelu(x, approximate=True)
def _silu(x):
    return jax.nn.silu(x)
def _sigmoid(x):
    return jax.nn.sigmoid(x)
def _layernorm(x, axis=-1, eps=1e-5):
    m = jnp.mean(x, axis=axis, keepdims=True)
    v = jnp.var(x, axis=axis, keepdims=True)
    return (x - m) / jnp.sqrt(v + eps)
def _scatter_add(tgt, idx, src, axis=0):
    return tgt.at[idx].add(src)
def _segment_sum(src, seg, n):
    return jax.ops.segment_sum(src, seg, n)
class _Rng:
    def __init__(self, key):
        self._k = key
    def _next(self):
        self._k, sub = jax.random.split(self._k)
        return sub
    def normal(self, shape):
        return jax.random.normal(self._next(), shape, dtype=jnp.bfloat16)
    def randint(self, lo, hi, shape):
        return jax.random.randint(self._next(), shape, lo, hi, dtype=jnp.int32)
    def uniform(self, shape, lo=0.0, hi=1.0):
        return jax.random.uniform(self._next(), shape, jnp.bfloat16, lo, hi)
    def permutation(self, n):
        return jax.random.permutation(self._next(), n)


kernel_name = 'standalone__gqa_block_cached__near_ridge'

def setup_inputs():
    _rng = _Rng(jax.random.key(int.from_bytes(__import__("os").urandom(4), "little")))
    _w = (lambda a: (lambda t: t.astype(jnp.bfloat16) if jnp.issubdtype(t.dtype, jnp.floating) else t)(jnp.asarray(a)))
    B, Sq, D = 8, 96, 640
    Hq, Hkv, Sk, Dh = 32, 32, 512, 128
    assert Hq % Hkv == 0, (Hq, Hkv)
    return {
        "x": _w((lambda *s: _rng.normal(s) * 0.2)(B, Sq, D)),
        "k_cache": _w((lambda *s: _rng.normal(s) * 3.2)(B, Hkv, Sk, Dh)),
        "v_cache": _w((lambda *s: _rng.normal(s) * 0.05)(B, Hkv, Sk, Dh)),
        "wq": _w((lambda *s: _rng.normal(s) * 0.2)(D, Hq * Dh) * (D ** -0.5)),
        "wo": _w((lambda *s: _rng.normal(s) * 0.05)(Hq * Dh, D) * ((Hq * Dh) ** -0.5)),
    }

def reference(x, k_cache, v_cache, wq, wo):
    B, Sq, D = x.shape
    Hq, Dh = 32, 128
    Hkv = k_cache.shape[1]
    rep = Hq // Hkv
    q = (lambda x, *d: x.transpose(*d))((x @ wq).reshape(B, Sq, Hq, Dh), 0, 2, 1, 3)
    k = jnp.repeat(k_cache, rep, axis=1)
    v = jnp.repeat(v_cache, rep, axis=1)
    scores = jnp.einsum("bhqd,bhkd->bhqk", q, k) * (Dh ** -0.5)
    p = _softmax(scores, axis=-1)
    o = jnp.einsum("bhqk,bhkd->bhqd", p, v)
    return (lambda x, *d: x.transpose(*d))(o, 0, 2, 1, 3).reshape(B, Sq, Hq * Dh) @ wo
```

```python
import jax
import jax.numpy as jnp
import jax.experimental.pallas as pl
import jax.experimental.pallas.tpu as pltpu

_LOG2E = 1.4426950408889634
_LANES = 128
_LOOKAHEAD = 2
_TAIL = (4, 2, 1, 1)


@jax.jit
def pallas_standalone__gqa_block_cached__near_ridge_kernel(
    x: jax.Array,
    k_cache: jax.Array,
    v_cache: jax.Array,
    wq: jax.Array,
    wo: jax.Array,
):
    B, Sq, D = x.shape
    _, H, Sk, Dh = k_cache.shape
    assert wq.shape == (D, H * Dh) and wo.shape == (H * Dh, D)
    assert v_cache.shape == k_cache.shape and Dh == _LANES
    assert D % _LANES == 0 and Sq % 16 == 0 and sum(_TAIL) == B
    M = B * Sq
    ND = D // _LANES
    L = _LOOKAHEAD
    R = L + 1
    NT = len(_TAIL)
    u32, bf16, f32 = jnp.uint32, jnp.bfloat16, jnp.float32
    nt_dims = (((1,), (1,)), ((), ()))
    qscale = Dh ** -0.5 * _LOG2E
    toff = [sum(_TAIL[:i]) for i in range(NT)]

    def ld(ref32, idx):
        return pltpu.bitcast(ref32[idx], bf16)

    def kernel_function(x_hbm, k_hbm, v_hbm, wq_hbm, wo_hbm, o_hbm,
                        x_v, k_v, v_v, wq_v, wo_v, q_buf, p_buf, l_buf, o_buf, acc,
                        out_v, s_buf, sems):
        x32, k32, v32 = x_v.bitcast(u32), k_v.bitcast(u32), v_v.bitcast(u32)
        wq32, q32, o32, p32 = (wq_v.bitcast(u32), q_buf.bitcast(u32),
                               o_buf.bitcast(u32), p_buf.bitcast(u32))

        def mo(i):
            return i if isinstance(i, int) else pl.multiple_of(i, Dh)

        def cpk(h):
            return pltpu.make_async_copy(k_hbm.at[:, h], k_v.at[h], sems.at[h % R])

        def cpv(h):
            return pltpu.make_async_copy(v_hbm.at[:, h], v_v.at[h], sems.at[R + h % R])

        def cpq(h):
            return pltpu.make_async_copy(wq_hbm.at[:, pl.ds(mo(h * Dh), Dh)], wq_v.at[h],
                                         sems.at[2 * R + h % R])

        def cpo(h):
            return pltpu.make_async_copy(wo_hbm.at[pl.ds(mo(h * Dh), Dh), :], wo_v.at[h],
                                         sems.at[3 * R + h % R])

        def cpx(j):
            return pltpu.make_async_copy(x_hbm.at[:, pl.ds(j * _LANES, _LANES)], x_v.at[j],
                                         sems.at[4 * R])

        def cpt(i):
            sl = pl.ds(toff[i], _TAIL[i])
            return pltpu.make_async_copy(v_hbm.at[sl, H - 1], v_v.at[H - 1, sl],
                                         sems.at[4 * R + 2 + i])

        def cpout(i):
            sl = pl.ds(toff[i] * Sq, _TAIL[i] * Sq)
            return pltpu.make_async_copy(out_v.at[sl], o_hbm.at[sl], sems.at[4 * R + 1])

        def start_last():
            cpk(H - 1).start()
            cpo(H - 1).start()
            for i in range(NT):
                cpt(i).start()

        def start_group(h):
            def full():
                cpk(h).start()
                cpq(h + 1).start()
                cpv(h).start()
                cpo(h).start()
            if isinstance(h, int):
                full() if h < H - 1 else start_last()
            else:
                pl.when(h < H - 1)(full)
                pl.when(h == H - 1)(start_last)

        def qproj(h):
            r = None
            for j in range(ND):
                t = jnp.dot(ld(x32, j), ld(wq32, (h, pl.ds(j * 64, 64))),
                            preferred_element_type=f32)
                r = t if r is None else r + t
            q32[h % 2] = pltpu.bitcast((r * qscale).astype(bf16), u32)

        def softmax(b):
            s = s_buf[b]
            m = jnp.max(s, axis=-1, keepdims=True)
            p = jnp.exp2(s - m)
            l = jnp.sum(p, axis=-1, keepdims=True)
            r = pltpu.reciprocal(l, approx=True)
            r = r * (2.0 - l * r)
            p32[b] = pltpu.bitcast(p.astype(bf16), u32)
            l_buf[b] = jnp.broadcast_to(r, (Sq, _LANES))

        def pv(h, b):
            o = jnp.dot(ld(p32, b), ld(v32, (h, b)), preferred_element_type=f32)
            return (o * l_buf[b]).astype(bf16)

        def kphase(h, do_q=True):
            cpk(h).wait()
            if do_q:
                cpq(h + 1).wait()
            for b in range(B):
                q = ld(q32, (h % 2, pl.ds(b * (Sq // 2), Sq // 2)))
                s_buf[b] = jax.lax.dot_general(q, ld(k32, (h, b)), nt_dims,
                                               preferred_element_type=f32)
            if do_q:
                qproj(h + 1)
            for b in range(B):
                softmax(b)

        def vphase(h):
            cpv(h).wait()
            cpo(h).wait()
            for b in range(B):
                o32[pl.ds(b * (Sq // 2), Sq // 2), :] = pltpu.bitcast(pv(h, b), u32)
            acc[...] += jnp.dot(ld(o32, slice(None)), wo_v[h], preferred_element_type=f32)

        for j in range(ND):
            cpx(j).start()
        cpq(0).start()
        for h in range(L):
            start_group(h)
        acc[...] = jnp.zeros_like(acc)
        for j in range(ND):
            cpx(j).wait()
        cpq(0).wait()
        qproj(0)

        def body(h, carry):
            start_group(h + L)
            kphase(h)
            vphase(h)
            return carry

        jax.lax.fori_loop(0, H - 1, body, 0)

        h = H - 1
        kphase(h, do_q=False)
        cpo(h).wait()
        for i in range(NT):
            cpt(i).wait()
            outs = [pv(h, b) for b in range(toff[i], toff[i] + _TAIL[i])]
            oo = jnp.concatenate(outs, axis=0) if len(outs) > 1 else outs[0]
            rows = pl.ds(toff[i] * Sq, _TAIL[i] * Sq)
            out_v[rows, :] = (acc[rows, :] + jnp.dot(oo, wo_v[h], preferred_element_type=f32)
                              ).astype(out_v.dtype)
            cpout(i).start()
        for i in range(NT):
            cpout(i).wait()

    any_spec = pl.BlockSpec(memory_space=pl.ANY)
    vmem = pltpu.VMEM
    out = pl.pallas_call(
        kernel_function,
        in_specs=[any_spec] * 5,
        out_specs=any_spec,
        out_shape=jax.ShapeDtypeStruct((M, D), x.dtype),
        scratch_shapes=[
            vmem((ND, M, _LANES), bf16),
            vmem((H, B, Sk, Dh), bf16),
            vmem((H, B, Sk, Dh), bf16),
            vmem((H, D, Dh), bf16),
            vmem((H, Dh, D), bf16),
            vmem((2, M, Dh), bf16),
            vmem((B, Sq, Sk), bf16),
            vmem((B, Sq, _LANES), f32),
            vmem((M, Dh), bf16),
            vmem((M, D), f32),
            vmem((M, D), x.dtype),
            vmem((B, Sq, Sk), f32),
            pltpu.SemaphoreType.DMA((4 * R + 2 + NT,)),
        ],
        compiler_params=pltpu.CompilerParams(vmem_limit_bytes=110 * 2**20),
    )(x.reshape(M, D), k_cache, v_cache, wq, wo)
    return out.reshape(B, Sq, D)
```

```python
import functools

import jax
import jax.numpy as jnp
import jax.experimental.pallas as pl
import jax.experimental.pallas.tpu as pltpu

_LOG2E = 1.4426950408889634
_LANES = 128
_HI, _LO = 0, 1
_CHUNK_ROWS = 128
_EARLY_B = 2
_LATE_B = 2
_TAIL = (4, 3, 1)


@jax.jit
def pallas_standalone__gqa_block_cached__near_ridge_kernel(
    x: jax.Array,
    k_cache: jax.Array,
    v_cache: jax.Array,
    wq: jax.Array,
    wo: jax.Array,
):
    B, Sq, D = x.shape
    _, H, Sk, Dh = k_cache.shape
    assert v_cache.shape == k_cache.shape and k_cache.shape[0] == B
    assert wq.shape == (D, H * Dh) and wo.shape == (H * Dh, D)
    assert (B, Sq, D, Sk, Dh) == (8, 96, 640, 512, 128) and H >= 4
    M = B * Sq
    ND = D // _LANES
    u32, bf16, f32 = jnp.uint32, jnp.bfloat16, jnp.float32
    nt_dims = (((1,), (1,)), ((), ()))
    qscale = Dh ** -0.5 * _LOG2E
    per_b = Sk // _CHUNK_ROWS
    n_early, n_late = _EARLY_B * per_b, _LATE_B * per_b
    assert n_early <= B and n_late <= B
    b_early = B - _EARLY_B
    b_late = b_early - _LATE_B
    o_q = o_o = H * B
    o_acc = H * B + 2
    n_acc = ND * B // 2
    SK0, SV0, SX, SO = 0, 2, 4, 5
    tail_sem = (SV0, SK0, SX)
    toff = [sum(_TAIL[:i]) for i in range(len(_TAIL))]
    assert sum(_TAIL) == B and (H - 1) % 2 == 1

    def ld(ref32, idx):
        return pltpu.bitcast(ref32[idx], bf16)

    def kernel_function(x_hbm, k_hbm, v_hbm, wq_hbm, wo_hbm, o_hbm,
                        av, ak, x_v, wq_v, wo_v, p_buf, l_buf, out_v, s_buf, sems):
        av32, ak32, akf = av.bitcast(u32), ak.bitcast(u32), ak.bitcast(f32)
        x32, wq32, p32 = x_v.bitcast(u32), wq_v.bitcast(u32), p_buf.bitcast(u32)

        def mo(i):
            return i if isinstance(i, int) else pl.multiple_of(i, Dh)

        def when(cond, fn):
            if isinstance(cond, (bool, int)):
                if cond:
                    fn()
            else:
                pl.when(cond)(fn)

        def q_idx(b):
            return (o_q + b // 4, pl.ds(64 * (b % 4), Sq // 2))

        def o_idx(b):
            return (o_o + b // 4, pl.ds(64 * (b % 4), Sq // 2))

        def acc_idx(j, b):
            return (o_acc + (j * B + b) // 2, pl.ds(128 * ((j * B + b) % 2), Sq))

        def sem_k(h):
            return SK0 + h % 2

        def sem_v(h):
            return SV0 + h % 2

        def cp_batches(src, dst, h, b0, nb, sem):
            return pltpu.make_async_copy(src.at[pl.ds(b0, nb), h], dst.at[pl.ds(h * B + b0, nb)],
                                         sems.at[sem])

        def cp_piece(src, dst, h, b0, c, sem):
            b, rows = b0 + c // per_b, pl.ds((c % per_b) * _CHUNK_ROWS, _CHUNK_ROWS)
            return pltpu.make_async_copy(src.at[b, h, rows], dst.at[h * B + b, rows],
                                         sems.at[sem])

        def cp_wq(h):
            return pltpu.make_async_copy(wq_hbm.at[:, pl.ds(mo(h * Dh), Dh)], wq_v.at[h],
                                         sems.at[sem_k(h - 1)])

        def cp_wo(h):
            return pltpu.make_async_copy(wo_hbm.at[pl.ds(mo(h * Dh), Dh), :], wo_v.at[h],
                                         sems.at[sem_v(h)])

        def cp_x(j):
            return pltpu.make_async_copy(x_hbm.at[:, pl.ds(j * _LANES, _LANES)], x_v.at[j],
                                         sems.at[SX])

        def cp_wq0():
            return pltpu.make_async_copy(wq_hbm.at[:, pl.ds(0, Dh)], wq_v.at[0], sems.at[SX])

        def cp_tail(i):
            return cp_batches(v_hbm, av, H - 1, toff[i], _TAIL[i], tail_sem[i])

        def cp_out(b0, nb):
            rows = pl.ds(b0 * Sq, nb * Sq)
            return pltpu.make_async_copy(out_v.at[rows], o_hbm.at[rows], sems.at[SO])

        def k_tick(h, t):
            if t < n_early:
                cp_piece(v_hbm, av, h, b_early, t, sem_v(h)).start(priority=_HI)
            elif B <= t < B + n_late:
                when(h + 1 < H - 1, lambda: cp_piece(
                    v_hbm, av, h + 1, b_late, t - B, sem_v(h + 1)).start(priority=_HI))

        def v_tick(h, t):
            if t < n_early:
                cp_piece(k_hbm, ak, h + 1, b_early, t, sem_k(h + 1)).start(priority=_HI)
            elif B <= t < B + n_late:
                when(h + 2 < H - 1, lambda: cp_piece(
                    k_hbm, ak, h + 2, b_late, t - B, sem_k(h + 2)).start(priority=_HI))

        def q_proj(h, tick=None):
            w = ld(wq32, (h, pl.ds((ND - 1) * 64, 64)))
            r = jnp.concatenate(
                [jnp.dot(ld(x32, (ND - 1, pl.ds(i * M // 8, M // 8))), w,
                         preferred_element_type=f32) for i in range(4)], axis=0)
            for j in range(ND - 1):
                r = r + jnp.dot(ld(x32, j), ld(wq32, (h, pl.ds(j * 64, 64))),
                                preferred_element_type=f32)
            q = pltpu.bitcast((r * qscale).astype(bf16), u32)
            for b in range(B):
                if tick is not None:
                    tick(B + b)
                av32[q_idx(b)] = q[b * Sq // 2:(b + 1) * Sq // 2]

        def qk(h, b):
            s_buf[b] = jax.lax.dot_general(ld(av32, q_idx(b)), ld(ak32, h * B + b), nt_dims,
                                           preferred_element_type=f32)

        def softmax(b):
            s = s_buf[b]
            m = jnp.max(s, axis=-1, keepdims=True)
            p = jnp.exp2(s - m)
            l = jnp.sum(p, axis=-1, keepdims=True)
            r = pltpu.reciprocal(l, approx=True)
            r = r * (2.0 - l * r)
            p32[b] = pltpu.bitcast(p.astype(bf16), u32)
            l_buf[b] = jnp.broadcast_to(r, (Sq, _LANES))

        def pv(h, b):
            o = jnp.dot(ld(p32, b), ld(av32, h * B + b), preferred_element_type=f32)
            return (o * l_buf[b]).astype(bf16)

        def k_phase(h):
            cp_batches(k_hbm, ak, h, 0, B, sem_k(h)).wait()
            cp_wq(h + 1).wait()
            full = jnp.logical_or(h == 0, h + 1 == H - 1)
            when(full, lambda: cp_batches(
                k_hbm, ak, h + 1, 0, b_early, sem_k(h + 1)).start(priority=_LO))
            when(jnp.logical_not(full), lambda: cp_batches(
                k_hbm, ak, h + 1, 0, b_late, sem_k(h + 1)).start(priority=_LO))
            when(h + 2 < H, lambda: cp_wq(h + 2).start(priority=_LO))
            tick = functools.partial(k_tick, h)
            for b in range(B):
                tick(b)
                qk(h, b)
            q_proj(h + 1, tick)
            for b in range(B):
                softmax(b)

        def v_phase(h):
            cp_batches(v_hbm, av, h, 0, B, sem_v(h)).wait()
            cp_wo(h).wait()

            def request_next():
                cp_batches(v_hbm, av, h + 1, 0, b_late, sem_v(h + 1)).start(priority=_LO)
                cp_wo(h + 1).start(priority=_LO)

            def request_last():
                cp_wo(H - 1).start(priority=_LO)
                for i in range(len(_TAIL)):
                    cp_tail(i).start(priority=_LO)

            when(h + 1 < H - 1, request_next)
            when(h + 1 == H - 1, request_last)
            outs = []
            for b in range(B):
                o = pv(h, b)
                v_tick(h, b)
                ak32[o_idx(b)] = pltpu.bitcast(o, u32)
                outs.append(o)
            o = jnp.concatenate(outs, axis=0)
            c = jnp.dot(o, wo_v[h, :, 0:(ND - 1) * _LANES], preferred_element_type=f32)
            w = wo_v[h, :, (ND - 1) * _LANES:D]
            c_last = jnp.concatenate(
                [jnp.dot(o[i * M // 4:(i + 1) * M // 4], w, preferred_element_type=f32)
                 for i in range(4)], axis=0)
            for b in range(B):
                v_tick(h, B + b)
                for j in range(ND - 1):
                    akf[acc_idx(j, b)] += c[b * Sq:(b + 1) * Sq, j * _LANES:(j + 1) * _LANES]
            for b in range(B):
                akf[acc_idx(ND - 1, b)] += c_last[b * Sq:(b + 1) * Sq]

        for j in range(ND):
            cp_x(j).start(priority=_LO)
        cp_wq0().start(priority=_LO)
        cp_batches(k_hbm, ak, 0, 0, B, sem_k(0)).start(priority=_LO)
        cp_wq(1).start(priority=_LO)
        cp_batches(v_hbm, av, 0, 0, b_early, sem_v(0)).start(priority=_LO)
        cp_wo(0).start(priority=_LO)
        akf[pl.ds(o_acc, n_acc)] = jnp.zeros((n_acc, Sk // 2, _LANES), f32)
        for j in range(ND):
            cp_x(j).wait()
        cp_wq0().wait()
        q_proj(0)

        def body(h, carry):
            k_phase(h)
            v_phase(h)
            return carry

        jax.lax.fori_loop(0, H - 1, body, 0)

        h = H - 1
        written = []

        def finish(outs, b0, nb):
            o = jnp.concatenate(outs[b0:b0 + nb], axis=0) if nb > 1 else outs[b0]
            c = jnp.dot(o, wo_v[h], preferred_element_type=f32)
            for i in range(nb):
                for j in range(ND):
                    out_v[pl.ds((b0 + i) * Sq, Sq), pl.ds(j * _LANES, _LANES)] = (
                        akf[acc_idx(j, b0 + i)]
                        + c[i * Sq:(i + 1) * Sq, j * _LANES:(j + 1) * _LANES]).astype(out_v.dtype)
            cp_out(b0, nb).start(priority=_HI)
            written.append((b0, nb))

        cp_batches(k_hbm, ak, h, 0, B, sem_k(h)).wait()
        for b in range(B):
            qk(h, b)
        for b in range(6):
            softmax(b)
        cp_wo(h).wait()
        cp_tail(0).wait()
        softmax(6)
        softmax(7)
        outs = [pv(h, b) for b in range(4)]
        finish(outs, 0, 2)
        cp_tail(1).wait()
        finish(outs, 2, 2)
        outs += [pv(h, b) for b in range(4, 7)]
        finish(outs, 4, 2)
        cp_tail(2).wait()
        outs.append(pv(h, 7))
        finish(outs, 6, 1)
        finish(outs, 7, 1)
        for b0, nb in written:
            cp_out(b0, nb).wait()

    any_spec = pl.BlockSpec(memory_space=pl.ANY)
    vmem = pltpu.VMEM
    out = pl.pallas_call(
        kernel_function,
        in_specs=[any_spec] * 5,
        out_specs=any_spec,
        out_shape=jax.ShapeDtypeStruct((M, D), x.dtype),
        scratch_shapes=[
            vmem((H * B + 2, Sk, _LANES), bf16),
            vmem((H * B + 2 + n_acc, Sk, _LANES), bf16),
            vmem((ND, M, _LANES), bf16),
            vmem((H, D, Dh), bf16),
            vmem((H, Dh, D), bf16),
            vmem((B, Sq, Sk), bf16),
            vmem((B, Sq, _LANES), f32),
            vmem((M, D), x.dtype),
            vmem((B, Sq, Sk), f32),
            pltpu.SemaphoreType.DMA((6,)),
        ],
        compiler_params=pltpu.CompilerParams(vmem_limit_bytes=110 * 2**20),
    )(x.reshape(M, D), k_cache, v_cache, wq, wo)
    return out.reshape(B, Sq, D)
```

```python
import functools

import jax
import jax.numpy as jnp
import jax.experimental.pallas as pl
import jax.experimental.pallas.tpu as pltpu

_LOG2E = 1.4426950408889634
_LANES = 128
_HI, _LO = 0, 1
_ROWS = 128
_TICK_ORDER = (0, 4, 1, 5, 2, 6, 3, 7)
_TAIL = (4, 4)


@jax.jit
def pallas_standalone__gqa_block_cached__near_ridge_kernel(
    x: jax.Array,
    k_cache: jax.Array,
    v_cache: jax.Array,
    wq: jax.Array,
    wo: jax.Array,
):
    B, Sq, D = x.shape
    _, H, Sk, Dh = k_cache.shape
    assert v_cache.shape == k_cache.shape and k_cache.shape[0] == B
    assert wq.shape == (D, H * Dh) and wo.shape == (H * Dh, D)
    assert (B, Sq, D, Sk, Dh) == (8, 96, 640, 512, 128) and H >= 4
    M = B * Sq
    ND = D // _LANES
    u32, bf16, f32 = jnp.uint32, jnp.bfloat16, jnp.float32
    nt_dims = (((1,), (1,)), ((), ()))
    qscale = Dh ** -0.5 * _LOG2E
    r_early, r_late = Sk - _ROWS, Sk - 2 * _ROWS
    o_q = o_o = H * B
    o_acc = H * B + 2
    n_acc = ND * B // 2
    SK0, SV0, SX, SO = 0, 2, 4, 5
    tail_sem = (SV0, SK0)
    toff = [sum(_TAIL[:i]) for i in range(len(_TAIL))]
    assert sum(_TAIL) == B and (H - 1) % 2 == 1

    def ld(ref32, idx):
        return pltpu.bitcast(ref32[idx], bf16)

    def kernel_function(x_hbm, k_hbm, v_hbm, wq_hbm, wo_hbm, o_hbm,
                        av, ak, x_v, wq_v, wo_v, p_buf, l_buf, out_v, s_buf, sems):
        av32, ak32, akf = av.bitcast(u32), ak.bitcast(u32), ak.bitcast(f32)
        x32, wq32, p32 = x_v.bitcast(u32), wq_v.bitcast(u32), p_buf.bitcast(u32)

        def mo(i):
            return i if isinstance(i, int) else pl.multiple_of(i, Dh)

        def when(cond, fn):
            if isinstance(cond, (bool, int)):
                if cond:
                    fn()
            else:
                pl.when(cond)(fn)

        def q_idx(b):
            return (o_q + b // 4, pl.ds(64 * (b % 4), Sq // 2))

        def o_idx(b):
            return (o_o + b // 4, pl.ds(64 * (b % 4), Sq // 2))

        def acc_idx(j, b):
            return (o_acc + (j * B + b) // 2, pl.ds(128 * ((j * B + b) % 2), Sq))

        def sem_k(h):
            return SK0 + h % 2

        def sem_v(h):
            return SV0 + h % 2

        def cp_batches(src, dst, h, b0, nb, sem):
            return pltpu.make_async_copy(src.at[pl.ds(b0, nb), h], dst.at[pl.ds(h * B + b0, nb)],
                                         sems.at[sem])

        def cp_piece(src, dst, h, r0, t, sem):
            b, rows = _TICK_ORDER[t], pl.ds(r0, _ROWS)
            return pltpu.make_async_copy(src.at[b, h, rows], dst.at[h * B + b, rows],
                                         sems.at[sem])

        def start_rows(src, dst, h, r_end, sem):
            for r0 in range(0, r_end, _ROWS):
                rows = pl.ds(r0, _ROWS)
                pltpu.make_async_copy(src.at[:, h, rows], dst.at[pl.ds(h * B, B), rows],
                                      sems.at[sem]).start(priority=_LO)

        def cp_wq(h):
            return pltpu.make_async_copy(wq_hbm.at[:, pl.ds(mo(h * Dh), Dh)], wq_v.at[h],
                                         sems.at[sem_k(h - 1)])

        def cp_wo(h):
            return pltpu.make_async_copy(wo_hbm.at[pl.ds(mo(h * Dh), Dh), :], wo_v.at[h],
                                         sems.at[sem_v(h)])

        def cp_x(j):
            return pltpu.make_async_copy(x_hbm.at[:, pl.ds(j * _LANES, _LANES)], x_v.at[j],
                                         sems.at[SX])

        def cp_wq0():
            return pltpu.make_async_copy(wq_hbm.at[:, pl.ds(0, Dh)], wq_v.at[0], sems.at[SX])

        def cp_tail(i):
            return cp_batches(v_hbm, av, H - 1, toff[i], _TAIL[i], tail_sem[i])

        def cp_out(b0, nb):
            rows = pl.ds(b0 * Sq, nb * Sq)
            return pltpu.make_async_copy(out_v.at[rows], o_hbm.at[rows], sems.at[SO])

        def k_tick(h, t):
            if t < B:
                cp_piece(v_hbm, av, h, r_early, t, sem_v(h)).start(priority=_HI)
            else:
                when(h + 1 < H - 1, lambda: cp_piece(
                    v_hbm, av, h + 1, r_late, t - B, sem_v(h + 1)).start(priority=_HI))

        def v_tick(h, t):
            if t < B:
                cp_piece(k_hbm, ak, h + 1, r_early, t, sem_k(h + 1)).start(priority=_HI)
            else:
                when(h + 2 < H - 1, lambda: cp_piece(
                    k_hbm, ak, h + 2, r_late, t - B, sem_k(h + 2)).start(priority=_HI))

        def q_proj(h, tick=None):
            w = ld(wq32, (h, pl.ds((ND - 1) * 64, 64)))
            r = jnp.concatenate(
                [jnp.dot(ld(x32, (ND - 1, pl.ds(i * M // 8, M // 8))), w,
                         preferred_element_type=f32) for i in range(4)], axis=0)
            for j in range(ND - 1):
                r = r + jnp.dot(ld(x32, j), ld(wq32, (h, pl.ds(j * 64, 64))),
                                preferred_element_type=f32)
            q = pltpu.bitcast((r * qscale).astype(bf16), u32)
            for b in range(B):
                if tick is not None:
                    tick(B + b)
                av32[q_idx(b)] = q[b * Sq // 2:(b + 1) * Sq // 2]

        def qk(h, b):
            s_buf[b] = jax.lax.dot_general(ld(av32, q_idx(b)), ld(ak32, h * B + b), nt_dims,
                                           preferred_element_type=f32)

        def softmax(b):
            s = s_buf[b]
            m = jnp.max(s, axis=-1, keepdims=True)
            p = jnp.exp2(s - m)
            l = jnp.sum(p, axis=-1, keepdims=True)
            r = pltpu.reciprocal(l, approx=True)
            r = r * (2.0 - l * r)
            p32[b] = pltpu.bitcast(p.astype(bf16), u32)
            l_buf[b] = jnp.broadcast_to(r, (Sq, _LANES))

        def pv(h, b):
            o = jnp.dot(ld(p32, b), ld(av32, h * B + b), preferred_element_type=f32)
            return (o * l_buf[b]).astype(bf16)

        def o_proj(h, o, rows_per_split):
            c = jnp.dot(o, wo_v[h, :, 0:(ND - 1) * _LANES], preferred_element_type=f32)
            w = wo_v[h, :, (ND - 1) * _LANES:D]
            c_last = jnp.concatenate(
                [jnp.dot(o[r0:r0 + rows_per_split], w, preferred_element_type=f32)
                 for r0 in range(0, o.shape[0], rows_per_split)], axis=0)
            return [c[:, j * _LANES:(j + 1) * _LANES] for j in range(ND - 1)] + [c_last]

        def k_phase(h):
            cp_batches(k_hbm, ak, h, 0, B, sem_k(h)).wait()
            cp_wq(h + 1).wait()
            full = jnp.logical_or(h == 0, h + 1 == H - 1)
            when(full, lambda: start_rows(k_hbm, ak, h + 1, r_early, sem_k(h + 1)))
            when(jnp.logical_not(full), lambda: start_rows(k_hbm, ak, h + 1, r_late, sem_k(h + 1)))
            when(h + 2 < H, lambda: cp_wq(h + 2).start(priority=_LO))
            tick = functools.partial(k_tick, h)
            for b in range(B):
                tick(b)
                qk(h, b)
            q_proj(h + 1, tick)
            for b in range(B):
                softmax(b)

        def v_phase(h):
            cp_batches(v_hbm, av, h, 0, B, sem_v(h)).wait()
            cp_wo(h).wait()

            def request_next():
                start_rows(v_hbm, av, h + 1, r_late, sem_v(h + 1))
                cp_wo(h + 1).start(priority=_LO)

            def request_last():
                cp_wo(H - 1).start(priority=_LO)
                for i in range(len(_TAIL)):
                    cp_tail(i).start(priority=_LO)

            when(h + 1 < H - 1, request_next)
            when(h + 1 == H - 1, request_last)
            outs = []
            for b in range(B):
                o = pv(h, b)
                v_tick(h, b)
                ak32[o_idx(b)] = pltpu.bitcast(o, u32)
                outs.append(o)
            c = o_proj(h, jnp.concatenate(outs, axis=0), M // 4)
            for b in range(B):
                v_tick(h, B + b)
                for j in range(ND - 1):
                    akf[acc_idx(j, b)] += c[j][b * Sq:(b + 1) * Sq]
            for b in range(B):
                akf[acc_idx(ND - 1, b)] += c[ND - 1][b * Sq:(b + 1) * Sq]

        for j in range(ND):
            cp_x(j).start(priority=_LO)
        cp_wq0().start(priority=_LO)
        cp_batches(k_hbm, ak, 0, 0, B, sem_k(0)).start(priority=_LO)
        cp_wq(1).start(priority=_LO)
        start_rows(v_hbm, av, 0, r_early, sem_v(0))
        cp_wo(0).start(priority=_LO)
        akf[pl.ds(o_acc, n_acc)] = jnp.zeros((n_acc, Sk // 2, _LANES), f32)
        for j in range(ND):
            cp_x(j).wait()
        cp_wq0().wait()
        q_proj(0)

        def body(h, carry):
            k_phase(h)
            v_phase(h)
            return carry

        jax.lax.fori_loop(0, H - 1, body, 0)

        h = H - 1
        written = []

        def finish(outs, b0, nb):
            c = o_proj(h, jnp.concatenate(outs[b0:b0 + nb], axis=0), Sq // 2)
            for i in range(nb):
                for j in range(ND):
                    out_v[pl.ds((b0 + i) * Sq, Sq), pl.ds(j * _LANES, _LANES)] = (
                        akf[acc_idx(j, b0 + i)] + c[j][i * Sq:(i + 1) * Sq]).astype(out_v.dtype)
            cp_out(b0, nb).start(priority=_HI)
            written.append((b0, nb))

        cp_batches(k_hbm, ak, h, 0, B, sem_k(h)).wait()
        for b in range(B):
            qk(h, b)
        for b in range(6):
            softmax(b)
        cp_wo(h).wait()
        cp_tail(0).wait()
        outs = [pv(h, 0), pv(h, 1)]
        softmax(6)
        outs += [pv(h, 2), pv(h, 3)]
        softmax(7)
        finish(outs, 0, 2)
        finish(outs, 2, 2)
        cp_tail(1).wait()
        outs += [pv(h, 4), pv(h, 5)]
        finish(outs, 4, 2)
        outs += [pv(h, 6), pv(h, 7)]
        finish(outs, 6, 2)
        for b0, nb in written:
            cp_out(b0, nb).wait()

    any_spec = pl.BlockSpec(memory_space=pl.ANY)
    vmem = pltpu.VMEM
    out = pl.pallas_call(
        kernel_function,
        in_specs=[any_spec] * 5,
        out_specs=any_spec,
        out_shape=jax.ShapeDtypeStruct((M, D), x.dtype),
        scratch_shapes=[
            vmem((H * B + 2, Sk, _LANES), bf16),
            vmem((H * B + 2 + n_acc, Sk, _LANES), bf16),
            vmem((ND, M, _LANES), bf16),
            vmem((H, D, Dh), bf16),
            vmem((H, Dh, D), bf16),
            vmem((B, Sq, Sk), bf16),
            vmem((B, Sq, _LANES), f32),
            vmem((M, D), x.dtype),
            vmem((B, Sq, Sk), f32),
            pltpu.SemaphoreType.DMA((6,)),
        ],
        compiler_params=pltpu.CompilerParams(vmem_limit_bytes=110 * 2**20),
    )(x.reshape(M, D), k_cache, v_cache, wq, wo)
    return out.reshape(B, Sq, D)
```

```python
import functools

import jax
import jax.numpy as jnp
import jax.experimental.pallas as pl
import jax.experimental.pallas.tpu as pltpu

_LOG2E = 1.4426950408889634
_LANES = 128
_HI, _LO = 0, 1
_ROWS = 128
_TICK_ORDER = (0, 4, 1, 5, 2, 6, 3, 7)
_BULK_SEGS = (0, 2)
_LATE_SEG = 3
_EARLY_SEG = 1
_TAIL = (3, 3, 2)


@jax.jit
def pallas_standalone__gqa_block_cached__near_ridge_kernel(
    x: jax.Array,
    k_cache: jax.Array,
    v_cache: jax.Array,
    wq: jax.Array,
    wo: jax.Array,
):
    B, Sq, D = x.shape
    _, H, Sk, Dh = k_cache.shape
    assert v_cache.shape == k_cache.shape and k_cache.shape[0] == B
    assert wq.shape == (D, H * Dh) and wo.shape == (H * Dh, D)
    assert (B, Sq, D, Sk, Dh) == (8, 96, 640, 512, 128) and H >= 4 and H & (H - 1) == 0
    M = B * Sq
    ND = D // _LANES
    bf16, f32 = jnp.bfloat16, jnp.float32
    nt_dims = (((1,), (1,)), ((), ()))
    qscale = Dh ** -0.5 * _LOG2E
    assert sorted(_BULK_SEGS + (_LATE_SEG, _EARLY_SEG)) == list(range(Sk // _ROWS))
    o_q = o_o = H * B
    o_c = H * B + 2
    SK0, SV0, SIO = 0, 2, 4
    tail_sem = (SIO, SV0, SK0)
    toff = [sum(_TAIL[:i]) for i in range(len(_TAIL))]
    assert sum(_TAIL) == B and (H - 1) % 2 == 1

    def kernel_function(x_hbm, k_hbm, v_hbm, wq_hbm, wo_hbm, o_hbm,
                        av, ak, x_v, wq_v, wo_v, p_buf, l_buf, out_v, s_buf, acc, sems):
        def head(h):
            return h if isinstance(h, int) else jnp.bitwise_and(h, H - 1)

        def mo(i):
            return i if isinstance(i, int) else pl.multiple_of(i, Dh)

        def when(cond, fn):
            if isinstance(cond, (bool, int)):
                if cond:
                    fn()
            else:
                pl.when(cond)(fn)

        def q_idx(b):
            return (o_q + b // 4, pl.ds(_LANES * (b % 4), Sq))

        def o_idx(b):
            return (o_o + b // 4, pl.ds(_LANES * (b % 4), Sq))

        def sem_k(h):
            return SK0 + h % 2

        def sem_v(h):
            return SV0 + h % 2

        def cp_batches(src, dst, h, b0, nb, sem):
            h = head(h)
            return pltpu.make_async_copy(src.at[pl.ds(b0, nb), h], dst.at[pl.ds(h * B + b0, nb)],
                                         sems.at[sem])

        def cp_piece(src, dst, h, seg, t, sem):
            h, b, rows = head(h), _TICK_ORDER[t], pl.ds(seg * _ROWS, _ROWS)
            return pltpu.make_async_copy(src.at[b, h, rows], dst.at[h * B + b, rows],
                                         sems.at[sem])

        def start_bulk(src, dst, h, with_late, sem):
            h = head(h)
            for seg in _BULK_SEGS + ((_LATE_SEG,) if with_late else ()):
                rows = pl.ds(seg * _ROWS, _ROWS)
                pltpu.make_async_copy(src.at[:, h, rows], dst.at[pl.ds(h * B, B), rows],
                                      sems.at[sem]).start(priority=_LO)

        def cp_wq(h):
            return pltpu.make_async_copy(wq_hbm.at[:, pl.ds(mo(head(h) * Dh), Dh)],
                                         wq_v.at[head(h)], sems.at[sem_k(h - 1)])

        def cp_wo(h):
            return pltpu.make_async_copy(wo_hbm.at[pl.ds(mo(head(h) * Dh), Dh), :],
                                         wo_v.at[head(h)], sems.at[sem_v(h)])

        def cp_x(j):
            return pltpu.make_async_copy(x_hbm.at[:, pl.ds(j * _LANES, _LANES)], x_v.at[j],
                                         sems.at[SIO])

        def cp_wq0():
            return pltpu.make_async_copy(wq_hbm.at[:, pl.ds(0, Dh)], wq_v.at[0], sems.at[SIO])

        def cp_tail(i):
            return cp_batches(v_hbm, av, H - 1, toff[i], _TAIL[i], tail_sem[i])

        def cp_out(b0, nb):
            rows = pl.ds(b0 * Sq, nb * Sq)
            return pltpu.make_async_copy(out_v.at[rows], o_hbm.at[rows], sems.at[SIO])

        def k_tick(h, t):
            if t < B:
                cp_piece(v_hbm, av, h, _EARLY_SEG, t, sem_v(h)).start(priority=_HI)
            else:
                when(h + 1 < H - 1, lambda: cp_piece(
                    v_hbm, av, h + 1, _LATE_SEG, t - B, sem_v(h + 1)).start(priority=_HI))

        def v_tick(h, t):
            if t < B:
                cp_piece(k_hbm, ak, h + 1, _EARLY_SEG, t, sem_k(h + 1)).start(priority=_HI)
            else:
                when(h + 2 < H - 1, lambda: cp_piece(
                    k_hbm, ak, h + 2, _LATE_SEG, t - B, sem_k(h + 2)).start(priority=_HI))

        def q_proj(h, tick=None):
            w = wq_v[h, pl.ds((ND - 1) * _LANES, _LANES)]
            r = jnp.concatenate(
                [jnp.dot(x_v[ND - 1, pl.ds(i * M // 4, M // 4)], w, preferred_element_type=f32)
                 for i in range(4)], axis=0)
            for j in range(ND - 1):
                r = r + jnp.dot(x_v[j], wq_v[h, pl.ds(j * _LANES, _LANES)],
                                preferred_element_type=f32)
            q = (r * qscale).astype(bf16)
            for b in range(B):
                if tick is not None:
                    tick(B + b)
                av[q_idx(b)] = q[b * Sq:(b + 1) * Sq]

        def qk(h, b):
            s_buf[b] = jax.lax.dot_general(av[q_idx(b)], ak[h * B + b], nt_dims,
                                           preferred_element_type=f32)

        def softmax(b):
            s = s_buf[b]
            m = jnp.max(s, axis=-1, keepdims=True)
            p = jnp.exp2(s - m)
            l = jnp.sum(p, axis=-1, keepdims=True)
            r = pltpu.reciprocal(l, approx=True)
            r = r * (2.0 - l * r)
            p_buf[b] = p.astype(bf16)
            l_buf[b] = jnp.broadcast_to(r, (Sq, _LANES))

        def pv(h, b):
            o = jnp.dot(p_buf[b], av[h * B + b], preferred_element_type=f32)
            return (o * l_buf[b]).astype(bf16)

        def o_proj(h, o, rows_per_split):
            c = jnp.dot(o, wo_v[h, :, 0:(ND - 1) * _LANES], preferred_element_type=f32)
            w = wo_v[h, :, (ND - 1) * _LANES:D]
            c_last = jnp.concatenate(
                [jnp.dot(o[r0:r0 + rows_per_split], w, preferred_element_type=f32)
                 for r0 in range(0, o.shape[0], rows_per_split)], axis=0)
            return [c[:, j * _LANES:(j + 1) * _LANES] for j in range(ND - 1)] + [c_last]

        def k_phase(h):
            cp_batches(k_hbm, ak, h, 0, B, sem_k(h)).wait()
            cp_wq(h + 1).wait()
            full = jnp.logical_or(h == 0, h + 1 == H - 1)
            when(full, lambda: start_bulk(k_hbm, ak, h + 1, True, sem_k(h + 1)))
            when(jnp.logical_not(full), lambda: start_bulk(k_hbm, ak, h + 1, False, sem_k(h + 1)))
            when(h + 2 < H, lambda: cp_wq(h + 2).start(priority=_LO))
            tick = functools.partial(k_tick, h)
            for b in range(B):
                tick(b)
                qk(h, b)
            q_proj(h + 1, tick)
            for b in range(B):
                softmax(b)

        def v_phase(h):
            cp_batches(v_hbm, av, h, 0, B, sem_v(h)).wait()
            cp_wo(h).wait()

            def request_next():
                start_bulk(v_hbm, av, h + 1, False, sem_v(h + 1))
                cp_wo(h + 1).start(priority=_LO)

            def request_last():
                cp_wo(H - 1).start(priority=_LO)
                for i in range(len(_TAIL)):
                    cp_tail(i).start(priority=_LO)

            when(h + 1 < H - 1, request_next)
            when(h + 1 == H - 1, request_last)
            outs = []
            for b in range(B):
                o = pv(h, b)
                v_tick(h, b)
                ak[o_idx(b)] = o
                outs.append(o)
            c = o_proj(h, jnp.concatenate(outs, axis=0), M // 4)
            for b in range(B):
                v_tick(h, B + b)
                ak[o_c, pl.ds(16 * b, 16)] = c[0][b * Sq:b * Sq + 16].astype(bf16)
                for j in range(ND - 1):
                    acc[j, pl.ds(b * Sq, Sq)] += c[j][b * Sq:(b + 1) * Sq]
            for b in range(B):
                acc[ND - 1, pl.ds(b * Sq, Sq)] += c[ND - 1][b * Sq:(b + 1) * Sq]

        for j in range(ND):
            cp_x(j).start(priority=_LO)
        cp_wq0().start(priority=_LO)
        cp_batches(k_hbm, ak, 0, 0, B, sem_k(0)).start(priority=_LO)
        cp_wq(1).start(priority=_LO)
        start_bulk(v_hbm, av, 0, True, sem_v(0))
        cp_wo(0).start(priority=_LO)
        acc[...] = jnp.zeros_like(acc)
        for j in range(ND):
            cp_x(j).wait()
        cp_wq0().wait()
        q_proj(0)

        def body(h, carry):
            k_phase(h)
            v_phase(h)
            return carry

        jax.lax.fori_loop(0, H - 1, body, 0)

        h = H - 1
        written = []

        def finish(outs, b0, nb):
            c = o_proj(h, jnp.concatenate(outs[b0:b0 + nb], axis=0), Sq // 2)
            for i in range(nb):
                for j in range(ND):
                    out_v[pl.ds((b0 + i) * Sq, Sq), pl.ds(j * _LANES, _LANES)] = (
                        acc[j, pl.ds((b0 + i) * Sq, Sq)] + c[j][i * Sq:(i + 1) * Sq]
                    ).astype(out_v.dtype)
            cp_out(b0, nb).start(priority=_HI)
            written.append((b0, nb))

        cp_batches(k_hbm, ak, h, 0, B, sem_k(h)).wait()
        for b in range(B):
            qk(h, b)
        for b in range(6):
            softmax(b)
        cp_wo(h).wait()
        cp_tail(0).wait()
        outs = [pv(h, 0), pv(h, 1)]
        softmax(6)
        softmax(7)
        outs.append(pv(h, 2))
        finish(outs, 0, 2)
        cp_tail(1).wait()
        outs.append(pv(h, 3))
        finish(outs, 2, 2)
        outs += [pv(h, 4), pv(h, 5)]
        finish(outs, 4, 2)
        cp_tail(2).wait()
        outs += [pv(h, 6), pv(h, 7)]
        finish(outs, 6, 1)
        finish(outs, 7, 1)
        for b0, nb in written:
            cp_out(b0, nb).wait()

    any_spec = pl.BlockSpec(memory_space=pl.ANY)
    vmem = pltpu.VMEM
    out = pl.pallas_call(
        kernel_function,
        in_specs=[any_spec] * 5,
        out_specs=any_spec,
        out_shape=jax.ShapeDtypeStruct((M, D), x.dtype),
        scratch_shapes=[
            vmem((H * B + 2, Sk, _LANES), bf16),
            vmem((H * B + 3, Sk, _LANES), bf16),
            vmem((ND, M, _LANES), bf16),
            vmem((H, D, Dh), bf16),
            vmem((H, Dh, D), bf16),
            vmem((B, Sq, Sk), bf16),
            vmem((B, Sq, _LANES), f32),
            vmem((M, D), x.dtype),
            vmem((B, Sq, Sk), f32),
            vmem((ND, M, _LANES), f32),
            pltpu.SemaphoreType.DMA((5,)),
        ],
        compiler_params=pltpu.CompilerParams(vmem_limit_bytes=110 * 2**20),
    )(x.reshape(M, D), k_cache, v_cache, wq, wo)
    return out.reshape(B, Sq, D)
```
